```python
import os as _os
_os.environ.setdefault('JAX_PLATFORMS', 'cpu')
import jax
import jax.numpy as jnp

def _softmax(x, axis=-1):
    return jax.nn.softmax(x, axis=axis)

def _gelu(x):
    return jax.nn.gelu(x, approximate=True)

def _silu(x):
    return jax.nn.silu(x)

def _sigmoid(x):
    return jax.nn.sigmoid(x)

def _layernorm(x, axis=-1, eps=1e-05):
    m = jnp.mean(x, axis=axis, keepdims=True)
    v = jnp.var(x, axis=axis, keepdims=True)
    return (x - m) / jnp.sqrt(v + eps)

def _scatter_add(tgt, idx, src, axis=0):
    return tgt.at[idx].add(src)

def _segment_sum(src, seg, n):
    return jax.ops.segment_sum(src, seg, n)

class _Rng:

    def __init__(self, key):
        self._k = key

    def _next(self):
        self._k, sub = jax.random.split(self._k)
        return sub

    def normal(self, shape):
        return jax.random.normal(self._next(), shape, dtype=jnp.bfloat16)

    def randint(self, lo, hi, shape):
        return jax.random.randint(self._next(), shape, lo, hi, dtype=jnp.int32)

    def uniform(self, shape, lo=0.0, hi=1.0):
        return jax.random.uniform(self._next(), shape, jnp.bfloat16, lo, hi)

    def permutation(self, n):
        return jax.random.permutation(self._next(), n)
kernel_name = 'adaLN_cond__sliding_local_dilated__dense_activation_relu__prompt'

def setup_inputs():
    _rng = _Rng(jax.random.key(int.from_bytes(__import__("os").urandom(4), "little")))
    _w = lambda a: (lambda t: t.astype(jnp.bfloat16) if jnp.issubdtype(t.dtype, jnp.floating) else t)(jnp.asarray(a))

    def _A_setup():
        B, S, D = (1, 2048, 576)
        return {'x': _w((lambda *s: _rng.normal(s) * 0.05)(B, S, D)), 'wqkv': _w((lambda *s: _rng.normal(s) * 0.05)(D, 3 * D)), 'wo': _w((lambda *s: _rng.normal(s) * 0.05)(D, D))}
    _A_in = _A_setup()

    def _B_setup():
        B, S, D, Dff = (1, 2048, 576, 4608)
        return {'x': _w((lambda *s: _rng.normal(s) * 0.05)(B, S, D)), 'w1': _w((lambda *s: _rng.normal(s) * 0.05)(D, Dff)), 'w2': _w((lambda *s: _rng.normal(s) * 0.05)(Dff, D))}
    _B_in = _B_setup()
    return {'A_x': _A_in['x'], 'A_wqkv': _A_in['wqkv'], 'A_wo': _A_in['wo'], 'B_x': _B_in['x'], 'B_w1': _B_in['w1'], 'B_w2': _B_in['w2'], 'c': _w((lambda *s: _rng.normal(s) * 0.05)(1, 576) * 8.0), 'w_mod': _w((lambda *s: _rng.normal(s) * 0.05)(576, 6 * 576) * 576 ** (-0.5) * 8.0)}

def reference(A_x, A_wqkv, A_wo, B_x, B_w1, B_w2, c, w_mod):

    def _A_ref(x, wqkv, wo):
        B, S, D = x.shape
        H = 32
        Dh = D // H
        W, dil = (8, 2)
        qkv = (lambda x, *d: x.transpose(*d))((x @ wqkv).reshape(B, S, 3, H, Dh), 2, 0, 3, 1, 4)
        q, k, v = (qkv[0], qkv[1], qkv[2])
        scale = Dh ** (-0.5)
        pos = jnp.arange(S)
        off = jnp.arange(W) * dil
        idx = pos[:, None] - off[None, :]
        mask = idx >= 0
        idx_c = jnp.where(mask, idx, 0).reshape(-1)
        kg = k[:, :, idx_c, :].reshape(B, H, S, W, Dh)
        vg = v[:, :, idx_c, :].reshape(B, H, S, W, Dh)
        logits = jnp.einsum('bhsd,bhswd->bhsw', q, kg) * scale
        logits = jnp.where(mask[None, None, :, :], logits, -1000000000.0)
        attn = _softmax(logits, axis=-1)
        o = jnp.einsum('bhsw,bhswd->bhsd', attn, vg)
        return (lambda x, *d: x.transpose(*d))(o, 0, 2, 1, 3).reshape(B, S, D) @ wo

    def _B_ref(x, w1, w2):
        h = jnp.einsum('bsd,df->bsf', x, w1)
        zero = jnp.zeros_like(h)
        h = jnp.maximum(h, zero)
        return jnp.einsum('bsf,fd->bsd', h, w2)
    x = A_x
    mod = (_silu(c) @ w_mod).reshape(c.shape[0], 6, 1, -1)
    sa, ca, ga, sb, cb, gb = (mod[:, 0].copy(), mod[:, 1].copy(), mod[:, 2].copy(), mod[:, 3].copy(), mod[:, 4].copy(), mod[:, 5].copy())
    h = _layernorm(x, axis=-1) * (1 + ca) + sa
    x = x + ga * _A_ref(h, A_wqkv, A_wo)
    h = _layernorm(x, axis=-1) * (1 + cb) + sb
    x = x + gb * _B_ref(h, B_w1, B_w2)
    return x
```

```python
import functools

import jax
import jax.numpy as jnp
import jax.experimental.pallas as pl
import jax.experimental.pallas.tpu as pltpu

_H = 32
_W = 8
_DIL = 2
_HALO = 16
_EPS = 1e-5
_NEG = -1000000000.0


def _kernel(x_ref, c_ref, wmod_ref, wqkv_ref, wo_ref, w1_ref, w2_ref, o_ref,
            mod_sc, wqkv_sc, wo_sc, k_sc, v_sc, *, T, D, DP, DH, FF_CHUNK):
    i = pl.program_id(0)
    f32 = jnp.float32
    bf16 = jnp.bfloat16

    @pl.when(i == 0)
    def _prologue():
        c = c_ref[...].astype(f32)
        sc = c * jax.nn.sigmoid(c)
        mod = jnp.dot(sc.astype(bf16), wmod_ref[...], preferred_element_type=f32)
        for j in range(6):
            mod_sc[j:j + 1, :] = mod[:, j * D:(j + 1) * D]
        r = jax.lax.broadcasted_iota(jnp.int32, (D, DP), 0)
        cidx = jax.lax.broadcasted_iota(jnp.int32, (D, DP), 1)
        perm = jnp.where(cidx == (r % DH) * _H + r // DH, 1.0, 0.0).astype(bf16)
        for j in range(3):
            wqkv_sc[:, j * DP:(j + 1) * DP] = jnp.dot(
                wqkv_ref[:, j * D:(j + 1) * D], perm,
                preferred_element_type=f32).astype(bf16)
        rt = jax.lax.broadcasted_iota(jnp.int32, (DP, D), 0)
        ct = jax.lax.broadcasted_iota(jnp.int32, (DP, D), 1)
        perm_t = jnp.where(rt == (ct % DH) * _H + ct // DH, 1.0, 0.0).astype(bf16)
        wo_sc[...] = jnp.dot(perm_t, wo_ref[...],
                             preferred_element_type=f32).astype(bf16)
        k_sc[0:_HALO, :] = jnp.zeros((_HALO, DP), f32)
        v_sc[0:_HALO, :] = jnp.zeros((_HALO, DP), f32)

    sa = mod_sc[0:1, :]
    ca = mod_sc[1:2, :]
    ga = mod_sc[2:3, :]
    sb = mod_sc[3:4, :]
    cb = mod_sc[4:5, :]
    gb = mod_sc[5:6, :]

    def layernorm(z):
        mu = jnp.mean(z, axis=-1, keepdims=True)
        zc = z - mu
        var = jnp.mean(zc * zc, axis=-1, keepdims=True)
        return zc * jax.lax.rsqrt(var + _EPS)

    x = x_ref[...].astype(f32)
    h = (layernorm(x) * (1.0 + ca) + sa).astype(bf16)
    qkv = jnp.dot(h, wqkv_sc[...], preferred_element_type=f32)
    scale = DH ** (-0.5)
    q = qkv[:, 0:DP] * scale
    k_sc[_HALO:_HALO + T, :] = qkv[:, DP:2 * DP]
    v_sc[_HALO:_HALO + T, :] = qkv[:, 2 * DP:3 * DP]

    nb = DP // 128
    pos = i * T + jax.lax.broadcasted_iota(jnp.int32, (T, 128), 0)
    logits = []
    for w in range(_W):
        ks = k_sc[_HALO - _DIL * w:_HALO - _DIL * w + T, :]
        p = q * ks
        s = p[:, 0:128]
        for b in range(1, nb):
            s = s + p[:, b * 128:(b + 1) * 128]
        s = s + pltpu.roll(s, 64, 1)
        s = s + pltpu.roll(s, 32, 1)
        if w > 0:
            s = jnp.where(pos >= _DIL * w, s, _NEG)
        logits.append(s)
    m = logits[0]
    for w in range(1, _W):
        m = jnp.maximum(m, logits[w])
    es = [jnp.exp(l - m) for l in logits]
    den = es[0]
    for w in range(1, _W):
        den = den + es[w]
    inv = 1.0 / den
    cols = []
    for b in range(nb):
        acc = None
        for w in range(_W):
            vs = v_sc[_HALO - _DIL * w:_HALO - _DIL * w + T, b * 128:(b + 1) * 128]
            t = es[w] * vs
            acc = t if acc is None else acc + t
        cols.append((acc * inv).astype(bf16))
    o = jnp.concatenate(cols, axis=1)

    k_sc[0:_HALO, :] = k_sc[T:T + _HALO, :]
    v_sc[0:_HALO, :] = v_sc[T:T + _HALO, :]

    x1 = x + ga * jnp.dot(o, wo_sc[...], preferred_element_type=f32)
    h2 = (layernorm(x1) * (1.0 + cb) + sb).astype(bf16)
    dff = w1_ref.shape[1]
    acc = None
    for j in range(dff // FF_CHUNK):
        a = jnp.dot(h2, w1_ref[:, j * FF_CHUNK:(j + 1) * FF_CHUNK],
                    preferred_element_type=f32)
        a = jnp.maximum(a, 0.0).astype(bf16)
        t = jnp.dot(a, w2_ref[j * FF_CHUNK:(j + 1) * FF_CHUNK, :],
                    preferred_element_type=f32)
        acc = t if acc is None else acc + t
    o_ref[...] = (x1 + gb * acc).astype(o_ref.dtype)


@jax.jit
def pallas_adaLN_cond__sliding_local_dilated__dense_activation_relu__prompt_kernel(
    A_x: jax.Array,
    A_wqkv: jax.Array,
    A_wo: jax.Array,
    B_x: jax.Array,
    B_w1: jax.Array,
    B_w2: jax.Array,
    c: jax.Array,
    w_mod: jax.Array,
):
    B, S, D = A_x.shape
    assert B == 1
    DH = D // _H
    DP = ((D + 127) // 128) * 128
    T = 256
    FF_CHUNK = 512
    dff = B_w1.shape[1]
    x2 = A_x.reshape(S, D)

    kern = functools.partial(_kernel, T=T, D=D, DP=DP, DH=DH, FF_CHUNK=FF_CHUNK)
    const = lambda i: (0, 0)
    one = pl.Buffered(1)
    out = pl.pallas_call(
        kern,
        grid=(S // T,),
        in_specs=[
            pl.BlockSpec((T, D), lambda i: (i, 0)),
            pl.BlockSpec((1, D), const, pipeline_mode=one),
            pl.BlockSpec((D, 6 * D), const, pipeline_mode=one),
            pl.BlockSpec((D, 3 * D), const, pipeline_mode=one),
            pl.BlockSpec((D, D), const, pipeline_mode=one),
            pl.BlockSpec((D, dff), const, pipeline_mode=one),
            pl.BlockSpec((dff, D), const, pipeline_mode=one),
        ],
        out_specs=pl.BlockSpec((T, D), lambda i: (i, 0)),
        out_shape=jax.ShapeDtypeStruct((S, D), A_x.dtype),
        scratch_shapes=[
            pltpu.VMEM((8, D), jnp.float32),
            pltpu.VMEM((D, 3 * DP), jnp.bfloat16),
            pltpu.VMEM((DP, D), jnp.bfloat16),
            pltpu.VMEM((T + _HALO, DP), jnp.float32),
            pltpu.VMEM((T + _HALO, DP), jnp.float32),
        ],
        compiler_params=pltpu.CompilerParams(
            dimension_semantics=("arbitrary",),
            vmem_limit_bytes=100 * 1024 * 1024,
        ),
    )(x2, c, w_mod, A_wqkv, A_wo, B_w1, B_w2)
    return out.reshape(B, S, D)
```

```python
import functools

import jax
import jax.numpy as jnp
import jax.experimental.pallas as pl
import jax.experimental.pallas.tpu as pltpu

_H = 32
_W = 8
_DIL = 2
_EPS = 1e-5
_NEG = -1000000000.0
_NT = (((1,), (1,)), ((), ()))
_TN = (((0,), (0,)), ((), ()))


def _kernel(xt_ref, c_ref, wmod_ref, wqkv_ref, wo_ref, w1_ref, w2t_ref, o_ref,
            mod_sc, wqkvt_sc, wot_sc, k_sc, v_sc, *, T, D, DH, FF_CHUNK):
    i = pl.program_id(0)
    f32 = jnp.float32
    bf16 = jnp.bfloat16
    nl = T // 128

    @pl.when(i == 0)
    def _prologue():
        c = c_ref[...].astype(f32)
        sc = c * jax.nn.sigmoid(c)
        mod = jnp.dot(sc.astype(bf16), wmod_ref[...], preferred_element_type=f32)
        mod_sc[...] = jnp.broadcast_to(mod, (128, 6 * D)).T
        r = jax.lax.broadcasted_iota(jnp.int32, (D, D), 0)
        n = jax.lax.broadcasted_iota(jnp.int32, (D, D), 1)
        pm = jnp.where(r == (n % DH) * _H + n // DH, 1.0, 0.0).astype(bf16)
        for j in range(3):
            wqkvt_sc[j * D:(j + 1) * D, :] = jax.lax.dot_general(
                pm, wqkv_ref[:, j * D:(j + 1) * D], _NT,
                preferred_element_type=f32).astype(bf16)
        wot_sc[...] = jax.lax.dot_general(
            wo_ref[...], pm, (((0,), (1,)), ((), ())),
            preferred_element_type=f32).astype(bf16)
        k_sc[:, 0:128] = jnp.zeros((D, 128), f32)
        v_sc[:, 0:128] = jnp.zeros((D, 128), f32)

    def modvec(j):
        return jnp.tile(mod_sc[j * D:(j + 1) * D, :], (1, nl))

    def layernorm(z):
        mu = jnp.mean(z, axis=0, keepdims=True)
        zc = z - mu
        var = jnp.mean(zc * zc, axis=0, keepdims=True)
        return zc * jax.lax.rsqrt(var + _EPS)

    x = xt_ref[...].astype(f32)
    h = (layernorm(x) * (1.0 + modvec(1)) + modvec(0)).astype(bf16)
    qkv = jnp.dot(wqkvt_sc[...], h, preferred_element_type=f32)
    scale = DH ** (-0.5)
    q = qkv[0:D, :] * scale
    k_sc[:, 128:128 + T] = qkv[D:2 * D, :]
    v_sc[:, 128:128 + T] = qkv[2 * D:3 * D, :]

    pos = i * T + jax.lax.broadcasted_iota(jnp.int32, (_H, T), 1)
    logits = []
    for w in range(_W):
        ks = k_sc[:, 128 - _DIL * w:128 - _DIL * w + T]
        p = q * ks
        s = p[0:_H, :]
        for d in range(1, DH):
            s = s + p[d * _H:(d + 1) * _H, :]
        if w > 0:
            s = jnp.where(pos >= _DIL * w, s, _NEG)
        logits.append(s)
    m = logits[0]
    for w in range(1, _W):
        m = jnp.maximum(m, logits[w])
    es = [jnp.exp(l - m) for l in logits]
    den = es[0]
    for w in range(1, _W):
        den = den + es[w]
    inv = 1.0 / den
    acc = None
    for w in range(_W):
        vs = v_sc[:, 128 - _DIL * w:128 - _DIL * w + T]
        t = jnp.tile(es[w], (DH, 1)) * vs
        acc = t if acc is None else acc + t
    o = (acc * jnp.tile(inv, (DH, 1))).astype(bf16)

    k_sc[:, 0:128] = k_sc[:, T:T + 128]
    v_sc[:, 0:128] = v_sc[:, T:T + 128]

    x1 = x + modvec(2) * jnp.dot(wot_sc[...], o, preferred_element_type=f32)
    h2 = (layernorm(x1) * (1.0 + modvec(4)) + modvec(3)).T.astype(bf16)
    dff = w1_ref.shape[1]
    acc = None
    for j in range(dff // FF_CHUNK):
        a = jnp.dot(h2, w1_ref[:, j * FF_CHUNK:(j + 1) * FF_CHUNK],
                    preferred_element_type=f32)
        a = jnp.maximum(a, 0.0).astype(bf16)
        t = jax.lax.dot_general(w2t_ref[:, j * FF_CHUNK:(j + 1) * FF_CHUNK], a, _NT,
                                preferred_element_type=f32)
        acc = t if acc is None else acc + t
    o_ref[...] = (x1 + modvec(5) * acc).astype(o_ref.dtype)


@jax.jit
def pallas_adaLN_cond__sliding_local_dilated__dense_activation_relu__prompt_kernel(
    A_x: jax.Array,
    A_wqkv: jax.Array,
    A_wo: jax.Array,
    B_x: jax.Array,
    B_w1: jax.Array,
    B_w2: jax.Array,
    c: jax.Array,
    w_mod: jax.Array,
):
    B, S, D = A_x.shape
    assert B == 1
    DH = D // _H
    T = 256
    FF_CHUNK = 512
    dff = B_w1.shape[1]
    xt = A_x.reshape(S, D).T
    w2t = B_w2.T

    kern = functools.partial(_kernel, T=T, D=D, DH=DH, FF_CHUNK=FF_CHUNK)
    const = lambda i: (0, 0)
    one = pl.Buffered(1)
    out = pl.pallas_call(
        kern,
        grid=(S // T,),
        in_specs=[
            pl.BlockSpec((D, T), lambda i: (0, i)),
            pl.BlockSpec((1, D), const, pipeline_mode=one),
            pl.BlockSpec((D, 6 * D), const, pipeline_mode=one),
            pl.BlockSpec((D, 3 * D), const, pipeline_mode=one),
            pl.BlockSpec((D, D), const, pipeline_mode=one),
            pl.BlockSpec((D, dff), const, pipeline_mode=one),
            pl.BlockSpec((D, dff), const, pipeline_mode=one),
        ],
        out_specs=pl.BlockSpec((D, T), lambda i: (0, i)),
        out_shape=jax.ShapeDtypeStruct((D, S), A_x.dtype),
        scratch_shapes=[
            pltpu.VMEM((6 * D, 128), jnp.float32),
            pltpu.VMEM((3 * D, D), jnp.bfloat16),
            pltpu.VMEM((D, D), jnp.bfloat16),
            pltpu.VMEM((D, T + 128), jnp.float32),
            pltpu.VMEM((D, T + 128), jnp.float32),
        ],
        compiler_params=pltpu.CompilerParams(
            dimension_semantics=("arbitrary",),
            vmem_limit_bytes=100 * 1024 * 1024,
        ),
    )(xt, c, w_mod, A_wqkv, A_wo, B_w1, w2t)
    return out.T.reshape(B, S, D)
```

```python
import functools

import jax
import jax.numpy as jnp
import jax.experimental.pallas as pl
import jax.experimental.pallas.tpu as pltpu

_H = 32
_W = 8
_DIL = 2
_HALO = 16
_EPS = 1e-5
_NEG = -1000000000.0
_NT = (((1,), (1,)), ((), ()))


def _kernel(xt_ref, xn_ref, c_ref, wmod_hbm, wqkv_ref, wo_ref, w1_hbm, w2t_hbm, o_ref,
            mod_sc, wqkv_sc, wot_sc, k_sc, v_sc, w1_sc, w2t_sc, wmod_sc, h_sc, sems,
            *, T, D, DP, DH, FF_CHUNK, NSTEPS):
    i = pl.program_id(0)
    f32 = jnp.float32
    bf16 = jnp.bfloat16
    nl = T // 128
    nb = DP // 128

    def modvec(j):
        return jnp.tile(mod_sc[j * D:(j + 1) * D, :], (1, nl))

    def layernorm(z):
        mu = jnp.mean(z, axis=0, keepdims=True)
        zc = z - mu
        var = jnp.mean(zc * zc, axis=0, keepdims=True)
        return zc * jax.lax.rsqrt(var + _EPS)

    def make_h(ref):
        z = ref[...].astype(f32)
        return (layernorm(z) * (1.0 + modvec(1)) + modvec(0)).T.astype(bf16)

    def w1_copy():
        return pltpu.make_async_copy(w1_hbm, w1_sc, sems.at[0])

    def w2_copy():
        return pltpu.make_async_copy(w2t_hbm, w2t_sc, sems.at[1])

    def wm_copy():
        return pltpu.make_async_copy(wmod_hbm, wmod_sc, sems.at[2])

    @pl.when(i == 0)
    def _prologue():
        wm_copy().start()
        w1_copy().start()
        w2_copy().start()
        n = jax.lax.broadcasted_iota(jnp.int32, (D, DP), 0)
        p = jax.lax.broadcasted_iota(jnp.int32, (D, DP), 1)
        pm = jnp.where(p == (n % DH) * _H + n // DH, 1.0, 0.0).astype(bf16)
        for j in range(3):
            wqkv_sc[:, j * DP:(j + 1) * DP] = jnp.dot(
                wqkv_ref[:, j * D:(j + 1) * D], pm,
                preferred_element_type=f32).astype(bf16)
        wot_sc[...] = jax.lax.dot_general(
            wo_ref[...], pm, (((0,), (0,)), ((), ())),
            preferred_element_type=f32).astype(bf16)
        wm_copy().wait()
        c = c_ref[...].astype(f32)
        sc = c * jax.nn.sigmoid(c)
        mod = jnp.dot(sc.astype(bf16), wmod_sc[...], preferred_element_type=f32)
        mod_sc[...] = jnp.broadcast_to(mod, (128, 6 * D)).T
        for b in range(nb):
            k_sc[b, 0:_HALO, :] = jnp.zeros((_HALO, 128), f32)
            v_sc[b, 0:_HALO, :] = jnp.zeros((_HALO, 128), f32)
        h_sc[...] = make_h(xt_ref)

    x = xt_ref[...].astype(f32)
    h = h_sc[...]
    qkv = jnp.dot(h, wqkv_sc[...], preferred_element_type=f32)
    scale = DH ** (-0.5)
    qb = [qkv[:, b * 128:(b + 1) * 128] * scale for b in range(nb)]
    for b in range(nb):
        k_sc[b, _HALO:_HALO + T, :] = qkv[:, DP + b * 128:DP + (b + 1) * 128]
        v_sc[b, _HALO:_HALO + T, :] = qkv[:, 2 * DP + b * 128:2 * DP + (b + 1) * 128]

    pos = i * T + jax.lax.broadcasted_iota(jnp.int32, (T, 128), 0)
    logits = []
    for w in range(_W):
        lo = _HALO - _DIL * w
        s = None
        for b in range(nb):
            t = qb[b] * k_sc[b, lo:lo + T, :]
            s = t if s is None else s + t
        s = s + pltpu.roll(s, 64, 1)
        s = s + pltpu.roll(s, 32, 1)
        if w > 0:
            s = jnp.where(pos >= _DIL * w, s, _NEG)
        logits.append(s)
    m = logits[0]
    for w in range(1, _W):
        m = jnp.maximum(m, logits[w])
    es = [jnp.exp(l - m) for l in logits]
    den = es[0]
    for w in range(1, _W):
        den = den + es[w]
    inv = 1.0 / den
    cols = []
    for b in range(nb):
        acc = None
        for w in range(_W):
            lo = _HALO - _DIL * w
            t = es[w] * v_sc[b, lo:lo + T, :]
            acc = t if acc is None else acc + t
        cols.append((acc * inv).astype(bf16))
    o = jnp.concatenate(cols, axis=1)

    for b in range(nb):
        k_sc[b, 0:_HALO, :] = k_sc[b, T:T + _HALO, :]
        v_sc[b, 0:_HALO, :] = v_sc[b, T:T + _HALO, :]

    y = jax.lax.dot_general(wot_sc[...], o, _NT, preferred_element_type=f32)
    x1 = x + modvec(2) * y
    h2 = (layernorm(x1) * (1.0 + modvec(4)) + modvec(3)).T.astype(bf16)

    @pl.when(i == 0)
    def _wait():
        w1_copy().wait()
        w2_copy().wait()

    dff = w1_sc.shape[1]
    acc = None
    for j in range(dff // FF_CHUNK):
        a = jnp.dot(h2, w1_sc[:, j * FF_CHUNK:(j + 1) * FF_CHUNK],
                    preferred_element_type=f32)
        a = jnp.maximum(a, 0.0).astype(bf16)
        t = jax.lax.dot_general(w2t_sc[:, j * FF_CHUNK:(j + 1) * FF_CHUNK], a, _NT,
                                preferred_element_type=f32)
        acc = t if acc is None else acc + t
    o_ref[...] = (x1 + modvec(5) * acc).astype(o_ref.dtype)
    h_sc[...] = make_h(xn_ref)


@jax.jit
def pallas_adaLN_cond__sliding_local_dilated__dense_activation_relu__prompt_kernel(
    A_x: jax.Array,
    A_wqkv: jax.Array,
    A_wo: jax.Array,
    B_x: jax.Array,
    B_w1: jax.Array,
    B_w2: jax.Array,
    c: jax.Array,
    w_mod: jax.Array,
):
    B, S, D = A_x.shape
    assert B == 1
    DH = D // _H
    DP = ((D + 127) // 128) * 128
    T = 256
    FF_CHUNK = 1536
    NSTEPS = S // T
    dff = B_w1.shape[1]
    xt = A_x.reshape(S, D).T
    w2t = B_w2.T

    kern = functools.partial(_kernel, T=T, D=D, DP=DP, DH=DH, FF_CHUNK=FF_CHUNK, NSTEPS=NSTEPS)
    const = lambda i: (0, 0)
    one = pl.Buffered(1)
    out = pl.pallas_call(
        kern,
        grid=(NSTEPS,),
        in_specs=[
            pl.BlockSpec((D, T), lambda i: (0, i)),
            pl.BlockSpec((D, T), lambda i: (0, jnp.minimum(i + 1, NSTEPS - 1))),
            pl.BlockSpec((1, D), const, pipeline_mode=one),
            pl.BlockSpec(memory_space=pl.ANY),
            pl.BlockSpec((D, 3 * D), const, pipeline_mode=one),
            pl.BlockSpec((D, D), const, pipeline_mode=one),
            pl.BlockSpec(memory_space=pl.ANY),
            pl.BlockSpec(memory_space=pl.ANY),
        ],
        out_specs=pl.BlockSpec((D, T), lambda i: (0, i)),
        out_shape=jax.ShapeDtypeStruct((D, S), A_x.dtype),
        scratch_shapes=[
            pltpu.VMEM((6 * D, 128), jnp.float32),
            pltpu.VMEM((D, 3 * DP), jnp.bfloat16),
            pltpu.VMEM((D, DP), jnp.bfloat16),
            pltpu.VMEM((DP // 128, T + _HALO, 128), jnp.float32),
            pltpu.VMEM((DP // 128, T + _HALO, 128), jnp.float32),
            pltpu.VMEM((D, dff), jnp.bfloat16),
            pltpu.VMEM((D, dff), jnp.bfloat16),
            pltpu.VMEM((D, 6 * D), jnp.bfloat16),
            pltpu.VMEM((T, D), jnp.bfloat16),
            pltpu.SemaphoreType.DMA((3,)),
        ],
        compiler_params=pltpu.CompilerParams(
            dimension_semantics=("arbitrary",),
            vmem_limit_bytes=100 * 1024 * 1024,
        ),
    )(xt, xt, c, w_mod, A_wqkv, A_wo, B_w1, w2t)
    return out.T.reshape(B, S, D)
```
